```python
import os as _os
_os.environ.setdefault("JAX_PLATFORMS", "cpu")
import jax
import jax.numpy as jnp

def _softmax(x, axis=-1):
    return jax.nn.softmax(x, axis=axis)
def _gelu(x):
    return jax.nn.gelu(x, approximate=True)
def _silu(x):
    return jax.nn.silu(x)
def _sigmoid(x):
    return jax.nn.sigmoid(x)
def _layernorm(x, axis=-1, eps=1e-5):
    m = jnp.mean(x, axis=axis, keepdims=True)
    v = jnp.var(x, axis=axis, keepdims=True)
    return (x - m) / jnp.sqrt(v + eps)
def _scatter_add(tgt, idx, src, axis=0):
    return tgt.at[idx].add(src)
def _segment_sum(src, seg, n):
    return jax.ops.segment_sum(src, seg, n)
class _Rng:
    def __init__(self, key):
        self._k = key
    def _next(self):
        self._k, sub = jax.random.split(self._k)
        return sub
    def normal(self, shape):
        return jax.random.normal(self._next(), shape, dtype=jnp.bfloat16)
    def randint(self, lo, hi, shape):
        return jax.random.randint(self._next(), shape, lo, hi, dtype=jnp.int32)
    def uniform(self, shape, lo=0.0, hi=1.0):
        return jax.random.uniform(self._next(), shape, jnp.bfloat16, lo, hi)
    def permutation(self, n):
        return jax.random.permutation(self._next(), n)


kernel_name = 'concat_heads__ssm_conv_s4__sliding_local_dilated__prompt'

def setup_inputs():
    _rng = _Rng(jax.random.key(int.from_bytes(__import__("os").urandom(4), "little")))
    _w = (lambda a: (lambda t: t.astype(jnp.bfloat16) if jnp.issubdtype(t.dtype, jnp.floating) else t)(jnp.asarray(a)))
    def _A_setup():
        B, L, D, N = 1, 2048, 640, 192
        A_re = -jnp.exp((lambda *s: _rng.normal(s) * 0.8)(D, N))
        A_im = jnp.pi * (lambda *s: _rng.normal(s) * 0.8)(D, N)
        B_re = (lambda *s: _rng.normal(s) * 0.8)(D, N)
        B_im = (lambda *s: _rng.normal(s) * 0.8)(D, N)
        C_re = (lambda *s: _rng.normal(s) * 0.8)(D, N)
        C_im = (lambda *s: _rng.normal(s) * 0.8)(D, N)
        log_dt = (lambda *s: _rng.normal(s) * 0.8)(D) * 0.5 - 4.0
        Dskip = (lambda *s: _rng.normal(s) * 0.05)(D)
        return {
            "u": _w((lambda *s: _rng.normal(s) * 0.05)(B, L, D)),
            "A_re": _w(A_re),
            "A_im": _w(A_im),
            "B_re": _w(B_re),
            "B_im": _w(B_im),
            "C_re": _w(C_re),
            "C_im": _w(C_im),
            "log_dt": _w(log_dt),
            "Dskip": _w(Dskip),
        }
    _A_in = _A_setup()

    def _B_setup():
        B, S, D = 1, 2048, 640
        return {
            "x": _w((lambda *s: _rng.normal(s) * 0.2)(B, S, D)),
            "wqkv": _w((lambda *s: _rng.normal(s) * 0.2)(D, 3 * D)),
            "wo": _w((lambda *s: _rng.normal(s) * 0.05)(D, D)),
        }
    _B_in = _B_setup()

    return {
        "A_u": _A_in["u"],
        "A_A_re": _A_in["A_re"],
        "A_A_im": _A_in["A_im"],
        "A_B_re": _A_in["B_re"],
        "A_B_im": _A_in["B_im"],
        "A_C_re": _A_in["C_re"],
        "A_C_im": _A_in["C_im"],
        "A_log_dt": _A_in["log_dt"],
        "A_Dskip": _A_in["Dskip"],
        "B_x": _B_in["x"],
        "B_wqkv": _B_in["wqkv"],
        "B_wo": _B_in["wo"],
    }

def reference(A_u, A_A_re, A_A_im, A_B_re, A_B_im, A_C_re, A_C_im, A_log_dt, A_Dskip, B_x, B_wqkv, B_wo):
    def _A_ref(u, A_re, A_im, B_re, B_im, C_re, C_im, log_dt, Dskip):
        Bsz, L, D = u.shape
        dt = jnp.exp(log_dt)[:, None]
        A = A_re + 1j * A_im
        Bc = B_re + 1j * B_im
        Cc = C_re + 1j * C_im
        logdA = dt * A
        dB = dt * Bc
        l = (lambda x, dt: x.astype(dt))(jnp.arange(L), A_re.dtype)
        P = jnp.exp(logdA[:, :, None] * l[None, None, :])
        K = jnp.einsum("dn,dnl,dn->dl", Cc, P, dB).real
        L2 = 2 * L
        Kp = jnp.pad(K, ((0, 0), (0, L)))
        up = (lambda x, *d: x.transpose(*d))(u, 0, 2, 1)
        up = jnp.pad(up, ((0, 0), (0, 0), (0, L)))
        Kf = (lambda x, axes=(-2,-1): jnp.fft.rfft2(x.astype(jnp.float32), axes=axes))(Kp[:, None, :], axes=(-2, -1))
        Uf = (lambda x, axes=(-2,-1): jnp.fft.rfft2(x.astype(jnp.float32), axes=axes))(up[:, :, None, :], axes=(-2, -1))
        Yf = Uf * Kf[None, :, :, :]
        y = (lambda x, s, axes=(-2,-1): jnp.fft.irfft2(x, s=s, axes=axes).astype(jnp.bfloat16))(Yf, (1, L2), axes=(-2, -1))[:, :, 0, :L]
        y = (lambda x, *d: x.transpose(*d))(y, 0, 2, 1) + u * Dskip[None, None, :]
        return y

    def _B_ref(x, wqkv, wo):
        B, S, D = x.shape
        H = 32; Dh = D // H
        W, dil = 8, 2
        qkv = (lambda x, *d: x.transpose(*d))((x @ wqkv).reshape(B, S, 3, H, Dh), 2, 0, 3, 1, 4)
        q, k, v = qkv[0], qkv[1], qkv[2]
        scale = Dh ** -0.5
        pos = jnp.arange(S)
        off = jnp.arange(W) * dil
        idx = pos[:, None] - off[None, :]
        mask = idx >= 0
        idx_c = jnp.where(mask, idx, 0).reshape(-1)
        kg = k[:, :, idx_c, :].reshape(B, H, S, W, Dh)
        vg = v[:, :, idx_c, :].reshape(B, H, S, W, Dh)
        logits = jnp.einsum("bhsd,bhswd->bhsw", q, kg) * scale
        logits = jnp.where(mask[None, None, :, :], logits, -1e9)
        attn = _softmax(logits, axis=-1)
        o = jnp.einsum("bhsw,bhswd->bhsd", attn, vg)
        return (lambda x, *d: x.transpose(*d))(o, 0, 2, 1, 3).reshape(B, S, D) @ wo

    a = _A_ref(A_u, A_A_re, A_A_im, A_B_re, A_B_im, A_C_re, A_C_im, A_log_dt, A_Dskip)
    b = _B_ref(B_x, B_wqkv, B_wo)
    return jnp.concatenate([a, b], axis=-1)
```

```python
import jax
import jax.numpy as jnp
import numpy as np
from jax import lax
from jax.experimental import pallas as pl
from jax.experimental.pallas import tpu as pltpu

L = 2048
D = 640
N = 192
H = 32
DH = 20
WIN, DIL = 8, 2
T = 128
NB = L // T
NT = D // 128
RB = 256
HALO = 16
KB = 5
CG = 4
MM = 128
MO = 64

F32, BF16 = jnp.float32, jnp.bfloat16
LOG2E = 1.4426950408889634

_A_PAIRS = [(1, 5), (2, 6), (3, 7), (4, 8),
            (258, 516), (260, 520), (262, 772), (264, 776),
            (1032, 1288), (1544, 1800)]
_LAST = lambda lane: lane == 127
_LOW = lambda lane: (lane & 2) == 0
_LOW_EVEN = lambda lane: (lane & 6) == 0
_G_TILES = ([(0, 0, None), (1, 1, None), (1, 2, _LAST), (2, 2, None), (3, 2, _LOW_EVEN),
             (3, 2, _LOW), (3, 3, None), (3, 3, None), (4, 3, _LOW), (4, 3, _LOW)]
            + [(4, 4, None)] * 6)
_SPLIT = 4


def _round_bf16(v):
    u = np.asarray(v, np.float32).view(np.uint32).astype(np.uint64)
    u = (u + 0x7FFF + ((u >> 16) & 1)) & 0xFFFF0000
    return u.astype(np.uint32).view(np.float32)


def _pack_rows(v):
    u = np.ascontiguousarray(_round_bf16(np.ascontiguousarray(v, np.float32))).view(np.uint32)
    return np.ascontiguousarray((u[..., 0::2, :] >> 16) | u[..., 1::2, :]).view(np.int32)


def _constants():
    bexp = np.array([8 * (j // 2) + 128 * (j % 2) for j in range(32)])
    lane = np.arange(128)
    b, s = lane // 4, lane % 4
    up = np.array([p[0] for p in _A_PAIRS])
    lo = np.array([p[1] for p in _A_PAIRS])
    t0 = np.where(b % 2 == 0, up[s], lo[s]) + 8 * (b // 2)
    t1 = t0 + 128
    t2 = up[4 + s] + bexp[b]
    t3 = lo[4 + s] + bexp[b]
    t4 = np.where(s < 2, up[8 + s % 2], lo[8 + s % 2]) + bexp[b]
    tiles = (t0, t1, t2, t3, t4)
    lr = _round_bf16(np.arange(L)).astype(np.int64)
    phi = 2 * np.pi * (np.r_[0:T:2, 1:T:2] + 0.5) / (2 * T)
    g = np.zeros((NB, 2 * T, 128))
    for j, (ta, tb, pick) in enumerate(_G_TILES):
        vals = np.where(pick(lane), tiles[ta], tiles[tb]) if pick else tiles[ta]
        where = {int(v): i for i, v in enumerate(vals)}
        lags = (range(1, T + 1) if j < _SPLIT - 1 else
                range(1, T) if j < _SPLIT else range(-T + 1, T))
        for off in lags:
            col = where[int(lr[T * j + off])]
            g[j, :T, col] += np.cos(phi * off)
            g[j, T:, col] -= np.sin(phi * off)
    ang = phi[:, None] * np.arange(T)[None, :]
    fu = np.concatenate([np.cos(ang), -np.sin(ang)], axis=0)
    fi = (fu.T / T).reshape(T, 2, T // 8, 8).transpose(0, 2, 1, 3)
    fi = fi.reshape(T, 2, T).transpose(1, 0, 2)
    return _pack_rows(g), _pack_rows(fu), _pack_rows(fi)


_G, _FU, _FI = _constants()

_NT_DIMS = (((1,), (1,)), ((), ()))


def _cmul(a, b):
    return (a[0] * b[0] - a[1] * b[1], a[0] * b[1] + a[1] * b[0])


def _csq(a):
    return ((a[0] - a[1]) * (a[0] + a[1]), (a[0] + a[0]) * a[1])


def _iota(shape, axis):
    return lax.broadcasted_iota(jnp.int32, shape, axis)


def _bf16(a):
    return pltpu.bitcast(a, BF16)


def _pack(a, b):
    return jnp.concatenate([a, b], axis=0).astype(BF16)


def _lane_gather(x, idx):
    return jnp.take_along_axis(x, idx, axis=1, mode="promise_in_bounds")


def _weave(*streams):
    def pieces(stream):
        for fn, args, cost in stream:
            gen = fn(*args)
            if gen is None:
                yield cost
            else:
                yield from gen

    live = [[0.0, float(sum(c for _, _, c in st)), pieces(st)] for st in streams if st]
    while live:
        cur = min(live, key=lambda e: e[0] / e[1])
        cost = next(cur[2], None)
        if cost is None:
            live = [e for e in live if e is not cur]
        else:
            cur[0] += cost


def _cat(ref, idx, rows=slice(None)):
    if ref.dtype != jnp.int32:
        ref = ref.bitcast(jnp.int32)
    return jnp.concatenate([_bf16(ref[i, rows, :]) for i in idx], axis=1)


def _kernel(u_hbm, are_hbm, aim_hbm, bre_hbm, bim_hbm, cre_hbm, cim_hbm,
            ldt_hbm, dsk_hbm, x_hbm, wqkv_hbm, wo_hbm, g_hbm, fu_hbm, fi_hbm, one_ref,
            out_hbm,
            ldt_ref, dsk_ref, fu_ref, fi_ref, par_v, u_v, x_v, wraw_v, woraw_v, g_v, w_v, wo_v, wof_v, nat_v,
            seed_v, lhs_all, rhs_all, kd_v, q_v, k_v, v_v, e_v, p_v, o_v, acc_v, tmp_v,
            uh_v, ch0_v, ch1_v, yh0_v, yh1_v, ya_v, yb_v,
            in_sem, out_sem):
    def slabs(hbm, vm, r0, r1):
        return [(hbm.at[0, r0:r1, 128 * t:128 * t + 128], vm.at[t, r0:r1, :])
                for t in range(NT)]

    def params(c0, c1):
        return [(r.at[:, c0:c1], par_v.at[i, :, c0:c1]) for i, r in
                enumerate((are_hbm, aim_hbm, bre_hbm, bim_hbm, cre_hbm, cim_hbm))]

    def wqkv(p):
        return [(wqkv_hbm.at[:, 128 * t:128 * t + 128], wraw_v.at[t])
                for t in range(NT * p, NT * p + NT)]

    groups = [[pltpu.make_async_copy(src, dst, in_sem.at[i]) for src, dst in grp]
              for i, grp in enumerate((
                  wqkv(0),
                  slabs(x_hbm, x_v, 0, RB),
                  wqkv(1),
                  params(0, 128) + [(ldt_hbm, ldt_ref), (dsk_hbm, dsk_ref)],
                  wqkv(2),
                  params(128, D),
                  slabs(x_hbm, x_v, RB, 2 * RB) + slabs(u_hbm, u_v, 0, RB) + [(fu_hbm, fu_ref)],
                  slabs(x_hbm, x_v, 2 * RB, L) + slabs(u_hbm, u_v, RB, L),
                  [(wo_hbm, woraw_v), (g_hbm, g_v), (fi_hbm, fi_ref)]))]

    def start(copies):
        for c in copies:
            c.start()

    def wait(copies):
        for c in copies:
            c.wait()

    start(groups[0] + groups[1] + groups[2])

    one_trip = one_ref[0]

    def region(fn):
        lax.fori_loop(0, one_trip, lambda _, c: (fn(), c)[1], 0)

    u_w, x_w = u_v.bitcast(jnp.int32), x_v.bitcast(jnp.int32)
    lane = _iota((8, 128), 1)
    sub = _iota((8, 128), 0)
    upper = sub < 4
    left = lane < 64

    skip = [None] * NT

    def ssm_setup(t):
        cols = slice(128 * t, 128 * t + 128)
        are, aim, bre, bim, cre, cim = (par_v[i, :, cols].astype(F32) for i in range(6))
        d = jnp.exp(ldt_ref[...].astype(F32).reshape(1, D)[:, cols]).astype(BF16).astype(F32)
        dsk = dsk_ref[...].astype(F32).reshape(1, D)
        w = _cmul((cre, cim), (d * bre, d * bim))
        skip[t] = jnp.sum(w[0], axis=0, keepdims=True) + dsk[:, cols]
        first8 = (_iota((N - 128, 128), 1) & 8) == 0
        for i, (va, vb) in enumerate(((d * are, d * aim), w)):
            nat_v[2 * i, cols, :] = va[:128].T
            nat_v[2 * i + 1, cols, :] = vb[:128].T
            nat_v[4 + i, cols, :] = jnp.concatenate(
                [jnp.where(first8, va[128:], pltpu.roll(vb[128:], 8, 1)),
                 jnp.where(first8, pltpu.roll(va[128:], 120, 1), vb[128:])], axis=0).T

    def kgen_seeds(step, buf, c):
        r0 = pl.multiple_of(step * 16, 16)
        rows8 = [pl.ds(pl.multiple_of(r0 + 8 * i, 8), 8) for i in range(2)]

        def param(i):
            return nat_v[i, rows8[c], :] if c < 2 else nat_v[4 + i // 2, rows8[i % 2], :]

        def put(slot, hi, lo):
            for part in range(2):
                r = pltpu.roll(lo[part], 4, 0)
                seed_v[6 * buf + 2 * c, 2 * slot + part] = jnp.where(upper, hi[part], r)
                seed_v[6 * buf + 2 * c + 1, 2 * slot + part] = jnp.where(upper, r, hi[part])

        th = param(1)
        un, z = (jnp.cos(th), jnp.sin(th)), {}
        mag = param(0)
        for p in (1, 2, 4, 8, 16, 32, 64, 128):
            if p in (1, 2, 4, 8, 128):
                e = jnp.exp2(mag * (p * LOG2E))
                z[p] = (e * un[0], e * un[1])
            if p < 128:
                un = _csq(un)
        for part, (v0, v1) in enumerate(((1.0, z[128][0]), (0.0, -z[128][1]))):
            seed_v[6 * buf + 2 * c, part] = jnp.where(upper, v0, pltpu.roll(v1, 4, 0))
            seed_v[6 * buf + 2 * c + 1, part] = jnp.where(upper, v0, v1)
        b8 = (z[8][0], -z[8][1])
        put(1, b8, b8)
        w = (param(2), param(3))
        p1 = _cmul(w, z[1])
        put(2, p1, _cmul(p1, z[4]))
        put(3, z[1], z[1])
        put(5, z[2], z[4])
        z256 = _csq(z[128])
        put(6, z[4], z256)
        z512 = _csq(z256)
        put(8, z512, z512)
        q258 = _cmul(z[2], z256)
        q516 = _csq(q258)
        put(4, _cmul(w, q258), _cmul(w, q516))
        p1032 = _cmul(w, _csq(q516))
        put(7, p1032, _cmul(p1032, z256))

    def kgen_tables(buf, c, h):
        def seed(slot):
            return tuple(seed_v[6 * buf + 2 * c + h, 2 * slot + i] for i in range(2))

        def emit(ref, i, v0, v1):
            (re0, im0), (re1, im1) = v0, v1
            rows = pl.ds(16 * i, 16)
            if c < 2:
                ref[12 * buf + 3 * (2 * c + h), rows, :] = _pack(re0, re1)
                ref[12 * buf + 3 * (2 * c + h) + 1, rows, :] = _pack(im0, im1)
            else:
                im0, im1 = pltpu.roll(im0, 64, 1), pltpu.roll(im1, 64, 1)
                ref[12 * buf + 3 * h + 2, rows, :] = _pack(
                    jnp.where(left, re0, im0), jnp.where(left, re1, im1))
                ref[12 * buf + 3 * (2 + h) + 2, rows, :] = _pack(
                    jnp.where(left, im0, re0), jnp.where(left, im1, re1))

        for ref, first, n in ((rhs_all, 0, 8), (lhs_all, 2, 2)):
            v, m = seed(first), seed(first + 1)
            for i in range(n):
                v1 = _cmul(v, m)
                emit(ref, i, v, v1)
                if i + 1 < n:
                    v = _cmul(v1, m)
        v, m = seed(4), seed(6)
        v1 = _cmul(v, seed(5))
        emit(lhs_all, 2, v, v1)
        emit(lhs_all, 3, _cmul(v, m), _cmul(v1, m))
        v = seed(7)
        emit(lhs_all, 4, v, _cmul(v, seed(8)))

    def kgen_contract(step, buf):
        r0 = pl.multiple_of(step * 16, 16)
        diag = (lane & ~3) | (sub & 3)
        slot = lane & 3
        tiles = []
        for grp in range(2):
            w = []
            for h in range(2):
                idx = [12 * buf + 3 * (2 * grp + h) + i for i in range(3)]
                o = lax.dot_general(_cat(lhs_all, idx), _cat(rhs_all, idx), _NT_DIMS,
                                    preferred_element_type=F32)
                yield 60
                p = [_lane_gather(o[8 * i:8 * i + 8], diag) for i in range(10)]

                def sel4(v):
                    return jnp.where(slot < 2, jnp.where(slot == 0, v[0], v[1]),
                                     jnp.where(slot == 2, v[2], v[3]))
                w.append((sel4(p[0:4]), sel4(p[4:8]),
                          jnp.where((slot & 1) == 0, p[8], p[9])))
            hi = [jnp.where(upper, a, b) for a, b in zip(*w)]
            lo = [pltpu.roll(jnp.where(upper, b, a), 4, 0) for a, b in zip(*w)]
            even = (lane & 4) == 0
            tiles.append((
                jnp.where(even, hi[0], pltpu.roll(lo[0], 4, 1)),
                jnp.where(even, pltpu.roll(hi[0], 124, 1), lo[0]),
                hi[1], lo[1], jnp.where(slot < 2, hi[2], lo[2])))
        for t in range(5):
            kd_v[t, pl.ds(r0, 16), :] = _pack(tiles[0][t], tiles[1][t])

    def seeds(s0, *offs):
        return [(kgen_seeds, (jnp.minimum(s0 + i, D // 16 - 1), i % KB, c), 88)
                for i in offs for c in range(3)]

    def tables(*offs):
        return [(kgen_tables, (i % KB, c, h), 44)
                for i in offs for c in range(3) for h in range(2)]

    def contract(s0, *offs):
        return [(kgen_contract, (s0 + i, i % KB), 240) for i in offs]

    def u_dft(c, t):
        rows = pl.ds(pl.multiple_of(c * (T // 2), T // 2), T // 2)
        f = jnp.dot(_bf16(fu_ref[...]), _bf16(u_w[t, rows, :]), preferred_element_type=F32)
        uh_v[t, c, 0:2 * T, :] = f
        uh_v[t, c, 2 * T:3 * T, :] = f[:T] + f[T:]

    wraw_w = wraw_v.bitcast(jnp.int32)
    res5 = lane - 5 * ((lane * 205) >> 10)

    def reorder_qkv(j, p):
        col = ((lane & (H - 1)) * DH + 5 * (lane >> 5) + j) & 127
        for i in range(D // 16):
            rows = pl.ds(8 * i, 8)
            acc = wraw_w[NT * p, rows, :]
            for t in range(1, NT):
                acc = jnp.where(res5 == (j - 128 * t) % 5,
                                wraw_w[NT * p + t, rows, :], acc)
            w_v[NT * p + j, rows, :] = _lane_gather(acc, col)

    def reorder_out(t):
        wof_v[t] = woraw_v[:, 128 * t:128 * t + 128].astype(F32)
        for j in range(NT):
            for i in range(4):
                r = 128 * j + H * i
                wo_v[t, r:r + H, :] = wof_v[t, pl.ds(j + 5 * i, H, stride=DH), :].astype(BF16)

    def keep_halo(ref):
        for t in range(NT):
            ref[t, 0:HALO, :] = ref[t, RB:RB + HALO, :]

    def project(blk, p, m, first):
        ref, r0 = ((q_v, 0), (k_v, HALO), (v_v, HALO))[p]
        if p > 0 and m == 0 and not first:
            keep_halo(ref)
        rows = pl.ds(pl.multiple_of(blk * (RB // 2) + m * (MM // 2), MM // 2), MM // 2)
        dst = pl.ds(r0 + m * MM, MM)
        for t in range(NT):
            ref[t, dst, :] = jnp.dot(
                _cat(x_w, [4], rows), _bf16(w_v[NT * p + t, 256:320]),
                preferred_element_type=F32)
            yield MM // 4
        for t in range(NT):
            val = ref[t, dst, :] + jnp.dot(
                _cat(x_w, range(4), rows), _bf16(w_v[NT * p + t, 0:256]),
                preferred_element_type=F32)
            ref[t, dst, :] = val * (DH ** -0.5 * LOG2E) if p == 0 else val
            if p > 0 and first and m == 0:
                ref[t, 0:HALO, :] = jnp.broadcast_to(val[0:1], (HALO, 128))
            yield MM

    def projects(blk, p, first=False):
        return [(project, (blk, p, m, first), MM * 25 // 4) for m in range(RB // MM)]

    def logits(i, first):
        q = [q_v[t, 8 * i:8 * i + 8, :] for t in range(NT)]
        for w in range(WIN):
            a = HALO + 8 * i - DIL * w
            s = q[0] * k_v[0, a:a + 8, :]
            for t in range(1, NT):
                s = s + q[t] * k_v[t, a:a + 8, :]
            e_v[w, 8 * i:8 * i + 8, :] = jnp.where(
                sub >= DIL * w - 8 * i, s + pltpu.roll(s, 64, 1), -0.5e9 * LOG2E
            ) if first and 8 * i < DIL * w else s + pltpu.roll(s, 64, 1)

    def weights(i):
        lg = []
        for w in range(WIN):
            s = e_v[w, 8 * i:8 * i + 8, :]
            s = s + pltpu.roll(s, 32, 1)
            lg.append(s)
        m = lg[0]
        for s in lg[1:]:
            m = jnp.maximum(m, s)
        den = None
        for w in range(WIN):
            e = jnp.exp2(lg[w] - m)
            p_v[w, 8 * i:8 * i + 8, :] = e
            den = e if den is None else den + e
        p_v[WIN, 8 * i:8 * i + 8, :] = 1.0 / den

    def mix(blk, i):
        e = [p_v[w, 16 * i:16 * i + 16, :] for w in range(WIN + 1)]
        rows = pl.ds(pl.multiple_of(blk * RB + 16 * i, 16), 16)
        for t in range(NT):
            acc = None
            for w in range(WIN):
                a = HALO + 16 * i - DIL * w
                term = e[w] * v_v[t, a:a + 16, :]
                acc = term if acc is None else acc + term
            o_v[t, rows, :] = (acc * e[WIN]).astype(BF16)

    NI = RB // 16

    all_weights = [(weights, (i,), 1) for i in range(2 * NI)]

    def all_logits(first):
        return [(logits, (i, first), 1) for i in range(2 * NI)]

    def mixes(blk):
        return [(mix, (blk, i), 1) for i in range(NI)]

    def u_dfts(c):
        return [(u_dft, (c, t), 64) for t in range(NT)]

    def reorders(p):
        return [(reorder_qkv, (j, p), 1) for j in range(NT)]

    wait(groups[0])
    start(groups[3] + groups[4])
    _weave(reorders(0))
    wait(groups[1])
    _weave(projects(0, 0, True)[:1])
    wait(groups[2])
    start(groups[5])
    _weave(projects(0, 0, True)[1:], reorders(1))
    wait(groups[3] + groups[4])
    start(groups[6])
    _weave(projects(0, 1, True), reorders(2), [(ssm_setup, (0,), 300)] + seeds(0, 0, 1, 2, 3))
    wait(groups[5])
    start(groups[7])
    _weave(projects(0, 2, True), all_logits(True), tables(0, 1),
           [(ssm_setup, (t,), 1) for t in range(1, NT)])
    wait(groups[6])

    def attn_body(blk, carry):
        @pl.when(blk == 2)
        def _():
            wait(groups[7])
            start(groups[8])

        s0 = KB * (blk - 1)
        region(lambda: _weave(
            seeds(s0, 4, 5, 6) + tables(2, 3), all_weights,
            contract(s0, 0, 1) + projects(blk, 0), u_dfts(2 * blk - 2)))
        region(lambda: _weave(
            contract(s0, 2, 3) + projects(blk, 1), u_dfts(2 * blk - 1),
            seeds(s0, 7, 8) + tables(4), mixes(blk - 1)))
        _weave(contract(s0, 4) + projects(blk, 2), tables(5, 6), all_logits(False))
        return carry

    lax.fori_loop(1, L // RB, attn_body, 0)

    wait(groups[8])
    ch, yh = (ch0_v, ch1_v), (yh0_v, yh1_v)

    out_copies = []

    def write_out(part, t, r0=0, r1=L):
        c0 = D * part + 128 * t
        out_copies.append(pltpu.make_async_copy(
            (ya_v, yb_v)[part].at[t, r0:r1], out_hbm.at[0, r0:r1, c0:c0 + 128], out_sem))
        out_copies[-1].start()

    def k_dft(t, j):
        ta, tb, pick = _G_TILES[j]
        kd_w = kd_v.bitcast(jnp.int32)
        vals = kd_w[ta, 64 * t:64 * t + 64, :]
        if pick:
            vals = jnp.where(pick(_iota((64, 128), 1)), vals, kd_w[tb, 64 * t:64 * t + 64, :])
        f = lax.dot_general(_bf16(g_v[j]), _bf16(vals), _NT_DIMS, preferred_element_type=F32)
        if j < _SPLIT - 1:
            acc_v[j, 0:2 * T, :] = f
        re, im = f[:T], f[T:]
        if 0 < j < _SPLIT:
            h = T // 2
            re = jnp.concatenate([re[:h] - acc_v[j - 1, T:T + h, :],
                                  re[h:] + acc_v[j - 1, T + h:2 * T, :]], axis=0)
            im = jnp.concatenate([im[:h] + acc_v[j - 1, 0:h, :],
                                  im[h:] - acc_v[j - 1, h:T, :]], axis=0)
        ch[t % 2][j, 0:T, :] = re
        ch[t % 2][j, T:2 * T, :] = im - re
        ch[t % 2][j, 2 * T:3 * T, :] = im + re

    def block_conv(t, r):
        tmp = tmp_v.at[r % 2]
        nh = NB // 2
        for part in range(3):
            for phase, (pc, pu) in enumerate(((0, 2), (1, 0), (2, 1))):
                def fetch(get):
                    return [get(2 * c + part) if part < 2 else get(2 * c) + get(2 * c + 1)
                            for c in range(nh)]
                f = fetch(lambda c: ch[t % 2][c, pl.ds(T * pc + 8 * r, 8), :])
                g = fetch(lambda c: uh_v[t, c, pl.ds(T * pu + 8 * r, 8), :])
                for n0 in range(0, nh, CG):
                    acc = {n: tmp[0, 0, n] if phase else None for n in range(n0, n0 + CG)}
                    for j in range(n0 + CG):
                        for n in range(max(n0, j), n0 + CG):
                            term = f[j] * g[n - j]
                            acc[n] = (term if acc[n] is None else
                                      acc[n] - term if phase == 2 else acc[n] + term)
                    for n in acc:
                        if phase == 0:
                            tmp[0, 0, n] = acc[n]
                        elif part < 2:
                            tmp[phase, part, n] = acc[n]
                        else:
                            odd = acc[n] - tmp[phase, 0, n] - tmp[phase, 1, n]
                            even = tmp[phase, 0, n]
                            if n:
                                even = even + tmp[phase, 1, n - 1]
                            if phase == 1:
                                tmp[0, 1, n], tmp[0, 2, n] = even, odd
                            else:
                                rows = pl.ds(16 * r, 16)
                                yh[t % 2][2 * n, rows, :] = _pack(even, tmp[0, 1, n])
                                yh[t % 2][2 * n + 1, rows, :] = _pack(odd, tmp[0, 2, n])
                yield 17 if part < 2 else 27

    def inv_dft(t, c):
        y = jnp.dot(_cat(fi_ref, range(2)), _cat(yh[t % 2], [c]), preferred_element_type=F32)
        rows = pl.ds(T * c, T)
        ya_v[t, rows, :] = (y + u_v[t, rows, :].astype(F32) * skip[t]).astype(BF16)

    def out_proj(n):
        t, c = n // 4, n % 4
        wo_w = wo_v.bitcast(jnp.int32)
        for m in range(512 // MO):
            acc_v[4 + c, m * MO:(m + 1) * MO, :] = jnp.dot(
                _cat(o_v, [4], pl.ds(256 * c + m * MO // 2, MO // 2)),
                _bf16(wo_w[t, 256:320]), preferred_element_type=F32)
            yield MO // 4
        for m in range(512 // MO):
            yb_v[t, pl.ds(512 * c + m * MO, MO), :] = (
                acc_v[4 + c, m * MO:(m + 1) * MO, :] + jnp.dot(
                    _cat(o_v, range(4), pl.ds(256 * c + m * MO // 2, MO // 2)),
                    _bf16(wo_w[t, 0:256]), preferred_element_type=F32)).astype(BF16)
            yield MO

    def k_dfts(t, js):
        return [(k_dft, (t, j), 64) for j in js]

    s0 = KB * (L // RB - 1)
    region(lambda: _weave(
        contract(s0, 0, 1) + k_dfts(0, range(NB)), u_dfts(NB - 2) + u_dfts(NB - 1),
        seeds(s0, 4) + tables(2, 3), all_weights, [(reorder_out, (t,), 1) for t in range(NT)]))
    region(lambda: _weave(
        contract(s0, 2, 3) + [(out_proj, (n,), 640) for n in range(3)],
        tables(4), mixes(L // RB - 1)))
    _weave(contract(s0, 4) + [(out_proj, (3,), 640)])
    write_out(1, 0)
    plan = [(0, range(NB), range(4, 8)), (1, range(NB), range(8, 11)),
            (2, range(NB), range(11, 14)), (3, range(NB), range(14, 17)),
            (4, range(0, 10), range(17, 19)), (4, range(10, NB), range(19, 20))]
    for t, freqs, chunks in plan:
        head = freqs[0] == 0
        region(lambda: _weave(
            [(block_conv, (t, i), 183) for i in freqs],
            ([(inv_dft, (t - 1, c), 64) for c in range(NB)] if t > 0 and head else [])
            + [(out_proj, (n,), 640) for n in chunks],
            k_dfts(t + 1, range(NB)) if t + 1 < NT else []))
        if t > 0 and head:
            write_out(0, t - 1)
        for n in chunks:
            write_out(1, n // 4, 512 * (n % 4), 512 * (n % 4) + 512)
    for c in range(NB):
        inv_dft(NT - 1, c)
        if c % 4 == 3:
            write_out(0, NT - 1, T * (c - 3), T * (c + 1))
    wait(out_copies)


@jax.jit
def pallas_concat_heads__ssm_conv_s4__sliding_local_dilated__prompt_kernel(
    A_u: jax.Array,
    A_A_re: jax.Array,
    A_A_im: jax.Array,
    A_B_re: jax.Array,
    A_B_im: jax.Array,
    A_C_re: jax.Array,
    A_C_im: jax.Array,
    A_log_dt: jax.Array,
    A_Dskip: jax.Array,
    B_x: jax.Array,
    B_wqkv: jax.Array,
    B_wo: jax.Array,
):
    hbm = pl.BlockSpec(memory_space=pl.ANY)
    I32 = jnp.int32
    return pl.pallas_call(
        _kernel,
        out_shape=jax.ShapeDtypeStruct((1, L, 2 * D), BF16),
        in_specs=[hbm] * 15 + [pl.BlockSpec(memory_space=pltpu.SMEM)],
        out_specs=hbm,
        scratch_shapes=[
            pltpu.VMEM((D,), BF16),
            pltpu.VMEM((D,), BF16),
            pltpu.VMEM(_FU.shape, I32),
            pltpu.VMEM(_FI.shape, I32),
            pltpu.VMEM((6, N, D), BF16),
            pltpu.VMEM((NT, L, 128), BF16),
            pltpu.VMEM((NT, L, 128), BF16),
            pltpu.VMEM((3 * NT, D, 128), BF16),
            pltpu.VMEM((D, D), BF16),
            pltpu.VMEM(_G.shape, I32),
            pltpu.VMEM((3 * NT, D // 2, 128), I32),
            pltpu.VMEM((NT, D, 128), BF16),
            pltpu.VMEM((NT, D, 128), F32),
            pltpu.VMEM((6, D, 128), F32),
            pltpu.VMEM((KB * 6, 18, 8, 128), F32),
            pltpu.VMEM((KB * 12, 80, 128), BF16),
            pltpu.VMEM((KB * 12, 128, 128), BF16),
            pltpu.VMEM((5, D, 128), BF16),
            pltpu.VMEM((NT, RB, 128), F32),
            pltpu.VMEM((NT, HALO + RB, 128), F32),
            pltpu.VMEM((NT, HALO + RB, 128), F32),
            pltpu.VMEM((WIN, RB, 128), F32),
            pltpu.VMEM((WIN + 1, RB, 128), F32),
            pltpu.VMEM((NT, L, 128), BF16),
            pltpu.VMEM((8, 512, 128), F32),
            pltpu.VMEM((2, 3, 3, NB // 2, 8, 128), F32),
            pltpu.VMEM((NT, NB, 3 * T, 128), F32),
            pltpu.VMEM((NB, 3 * T, 128), F32),
            pltpu.VMEM((NB, 3 * T, 128), F32),
            pltpu.VMEM((NB, 2 * T, 128), BF16),
            pltpu.VMEM((NB, 2 * T, 128), BF16),
            pltpu.VMEM((NT, L, 128), BF16),
            pltpu.VMEM((NT, L, 128), BF16),
            pltpu.SemaphoreType.DMA((9,)),
            pltpu.SemaphoreType.DMA(()),
        ],
        compiler_params=pltpu.CompilerParams(vmem_limit_bytes=100 * 1024 * 1024),
        name="s4_attn",
    )(A_u, A_A_re.T, A_A_im.T, A_B_re.T, A_B_im.T, A_C_re.T, A_C_im.T,
      A_log_dt, A_Dskip, B_x, B_wqkv, B_wo, _G, _FU, _FI, np.ones((1,), np.int32))
```

```python
import jax
import jax.numpy as jnp
import numpy as np
from jax import lax
from jax.experimental import pallas as pl
from jax.experimental.pallas import tpu as pltpu

L = 2048
D = 640
N = 192
H = 32
DH = 20
WIN, DIL = 8, 2
T = 128
NB = L // T
NT = D // 128
RB = 512
HALO = 16
KB = 11
CG = 4
MM = 64

F32, BF16 = jnp.float32, jnp.bfloat16
LOG2E = 1.4426950408889634

_A_PAIRS = [(1, 5), (2, 6), (3, 7), (4, 8),
            (258, 516), (260, 520), (262, 772), (264, 776),
            (1032, 1288), (1544, 1800)]
_LAST = lambda lane: lane == 127
_LOW = lambda lane: (lane & 2) == 0
_LOW_EVEN = lambda lane: (lane & 6) == 0
_G_TILES = ([(0, 0, None), (1, 1, None), (1, 2, _LAST), (2, 2, None), (3, 2, _LOW_EVEN),
             (3, 2, _LOW), (3, 3, None), (3, 3, None), (4, 3, _LOW), (4, 3, _LOW)]
            + [(4, 4, None)] * 6)
_SPLIT = 4


def _round_bf16(v):
    u = np.asarray(v, np.float32).view(np.uint32).astype(np.uint64)
    u = (u + 0x7FFF + ((u >> 16) & 1)) & 0xFFFF0000
    return u.astype(np.uint32).view(np.float32)


def _pack_rows(v):
    u = np.ascontiguousarray(_round_bf16(np.ascontiguousarray(v, np.float32))).view(np.uint32)
    return np.ascontiguousarray((u[..., 0::2, :] >> 16) | u[..., 1::2, :]).view(np.int32)


def _constants():
    bexp = np.array([8 * (j // 2) + 128 * (j % 2) for j in range(32)])
    lane = np.arange(128)
    b, s = lane // 4, lane % 4
    up = np.array([p[0] for p in _A_PAIRS])
    lo = np.array([p[1] for p in _A_PAIRS])
    t0 = np.where(b % 2 == 0, up[s], lo[s]) + 8 * (b // 2)
    t1 = t0 + 128
    t2 = up[4 + s] + bexp[b]
    t3 = lo[4 + s] + bexp[b]
    t4 = np.where(s < 2, up[8 + s % 2], lo[8 + s % 2]) + bexp[b]
    tiles = (t0, t1, t2, t3, t4)
    lr = _round_bf16(np.arange(L)).astype(np.int64)
    phi = 2 * np.pi * (np.r_[0:T:2, 1:T:2] + 0.5) / (2 * T)
    g = np.zeros((NB, 2 * T, 128))
    for j, (ta, tb, pick) in enumerate(_G_TILES):
        vals = np.where(pick(lane), tiles[ta], tiles[tb]) if pick else tiles[ta]
        where = {int(v): i for i, v in enumerate(vals)}
        lags = (range(1, T + 1) if j < _SPLIT - 1 else
                range(1, T) if j < _SPLIT else range(-T + 1, T))
        for off in lags:
            col = where[int(lr[T * j + off])]
            g[j, :T, col] += np.cos(phi * off)
            g[j, T:, col] -= np.sin(phi * off)
    ang = phi[:, None] * np.arange(T)[None, :]
    fu = np.concatenate([np.cos(ang), -np.sin(ang)], axis=0)
    fi = (fu.T / T).reshape(T, 2, T // 8, 8).transpose(0, 2, 1, 3)
    fi = fi.reshape(T, 2, T).transpose(1, 0, 2)
    return _pack_rows(g), _pack_rows(fu), _pack_rows(fi)


_G, _FU, _FI = _constants()

_NT_DIMS = (((1,), (1,)), ((), ()))


def _cmul(a, b):
    return (a[0] * b[0] - a[1] * b[1], a[0] * b[1] + a[1] * b[0])


def _csq(a):
    return ((a[0] - a[1]) * (a[0] + a[1]), (a[0] + a[0]) * a[1])


def _iota(shape, axis):
    return lax.broadcasted_iota(jnp.int32, shape, axis)


def _bf16(a):
    return pltpu.bitcast(a, BF16)


def _pack(a, b):
    return jnp.concatenate([a, b], axis=0).astype(BF16)


def _lane_gather(x, idx):
    return jnp.take_along_axis(x, idx, axis=1, mode="promise_in_bounds")


def _weave(*streams):
    def pieces(stream):
        for fn, args, cost in stream:
            gen = fn(*args)
            if gen is None:
                yield cost
            else:
                yield from gen

    live = [[0.0, float(sum(c for _, _, c in st)), pieces(st)] for st in streams if st]
    while live:
        cur = min(live, key=lambda e: e[0] / e[1])
        cost = next(cur[2], None)
        if cost is None:
            live = [e for e in live if e is not cur]
        else:
            cur[0] += cost


def _cat(ref, idx, rows=slice(None)):
    if ref.dtype != jnp.int32:
        ref = ref.bitcast(jnp.int32)
    return jnp.concatenate([_bf16(ref[i, rows, :]) for i in idx], axis=1)


def _kernel(u_hbm, are_hbm, aim_hbm, bre_hbm, bim_hbm, cre_hbm, cim_hbm,
            ldt_hbm, dsk_hbm, x_hbm, wqkv_hbm, wo_hbm, g_hbm, fu_hbm, fi_hbm, one_ref,
            out_hbm,
            fu_ref, fi_ref, par_v, u_v, x_v, wraw_v, woraw_v, g_v, w_v, wo_v, wof_v, nat_v,
            seed_v, lhs_all, rhs_all, kd_v, q_v, k_v, v_v, e_v, p_v, o_v, acc_v, tmp_v,
            uh_v, ch0_v, ch1_v, yh0_v, yh1_v, ya_v, yb_v, skip_v, ldt_ref, dsk_ref,
            in_sem, out_sem):
    def slabs(hbm, vm, r0, r1):
        return [(hbm.at[0, r0:r1, 128 * t:128 * t + 128], vm.at[t, r0:r1, :])
                for t in range(NT)]

    def params(c0, c1):
        return [(r.at[:, c0:c1], par_v.at[i, :, c0:c1]) for i, r in
                enumerate((are_hbm, aim_hbm, bre_hbm, bim_hbm, cre_hbm, cim_hbm))]

    def wqkv(p):
        return [(wqkv_hbm.at[:, 128 * t:128 * t + 128], wraw_v.at[t])
                for t in range(NT * p, NT * p + NT)]

    groups = [[pltpu.make_async_copy(src, dst, in_sem.at[i]) for src, dst in grp]
              for i, grp in enumerate((
                  params(0, 128) + [(ldt_hbm, ldt_ref), (dsk_hbm, dsk_ref)],
                  wqkv(0),
                  slabs(x_hbm, x_v, 0, RB // 2),
                  slabs(x_hbm, x_v, RB // 2, RB),
                  wqkv(1),
                  wqkv(2),
                  params(128, D),
                  slabs(x_hbm, x_v, RB, 2 * RB) + slabs(u_hbm, u_v, 0, RB) + [(fu_hbm, fu_ref)],
                  slabs(x_hbm, x_v, 2 * RB, L) + slabs(u_hbm, u_v, RB, L),
                  [(wo_hbm, woraw_v), (g_hbm, g_v), (fi_hbm, fi_ref)]))]

    def start(copies):
        for c in copies:
            c.start()

    def wait(copies):
        for c in copies:
            c.wait()

    start(sum(groups[:9], []))

    one_trip = one_ref[0]

    def region(fn):
        lax.fori_loop(0, one_trip, lambda _, c: (fn(), c)[1], 0)

    u_w, x_w = u_v.bitcast(jnp.int32), x_v.bitcast(jnp.int32)
    lane = _iota((8, 128), 1)
    sub = _iota((8, 128), 0)
    upper = sub < 4
    left = lane < 64

    def ssm_setup(t):
        cols = slice(128 * t, 128 * t + 128)
        are, aim, bre, bim, cre, cim = (par_v[i, :, cols].astype(F32) for i in range(6))
        d = jnp.exp(ldt_ref[...].astype(F32).reshape(1, D)[:, cols]).astype(BF16).astype(F32)
        dsk = dsk_ref[...].astype(F32).reshape(1, D)
        w = _cmul((cre, cim), (d * bre, d * bim))
        skip_v[t] = jnp.sum(w[0], axis=0, keepdims=True) + dsk[:, cols]
        first8 = (_iota((N - 128, 128), 1) & 8) == 0
        for i, (va, vb) in enumerate(((d * are, d * aim), w)):
            nat_v[2 * i, cols, :] = va[:128].T
            nat_v[2 * i + 1, cols, :] = vb[:128].T
            nat_v[4 + i, cols, :] = jnp.concatenate(
                [jnp.where(first8, va[128:], pltpu.roll(vb[128:], 8, 1)),
                 jnp.where(first8, pltpu.roll(va[128:], 120, 1), vb[128:])], axis=0).T

    def kgen_seeds(step, buf, c):
        r0 = pl.multiple_of(step * 16, 16)
        rows8 = [pl.ds(pl.multiple_of(r0 + 8 * i, 8), 8) for i in range(2)]

        def param(i):
            return nat_v[i, rows8[c], :] if c < 2 else nat_v[4 + i // 2, rows8[i % 2], :]

        def put(slot, hi, lo):
            for part in range(2):
                r = pltpu.roll(lo[part], 4, 0)
                seed_v[6 * buf + 2 * c, 2 * slot + part] = jnp.where(upper, hi[part], r)
                seed_v[6 * buf + 2 * c + 1, 2 * slot + part] = jnp.where(upper, r, hi[part])

        th = param(1)
        un, z = (jnp.cos(th), jnp.sin(th)), {}
        yield 42
        mag = param(0)
        for p in (1, 2, 4, 8, 16, 32, 64, 128):
            if p in (1, 2, 4, 8, 128):
                e = jnp.exp2(mag * (p * LOG2E))
                z[p] = (e * un[0], e * un[1])
            if p < 128:
                un = _csq(un)
        for part, (v0, v1) in enumerate(((1.0, z[128][0]), (0.0, -z[128][1]))):
            seed_v[6 * buf + 2 * c, part] = jnp.where(upper, v0, pltpu.roll(v1, 4, 0))
            seed_v[6 * buf + 2 * c + 1, part] = jnp.where(upper, v0, v1)
        yield 14
        b8 = (z[8][0], -z[8][1])
        put(1, b8, b8)
        w = (param(2), param(3))
        p1 = _cmul(w, z[1])
        put(2, p1, _cmul(p1, z[4]))
        put(3, z[1], z[1])
        put(5, z[2], z[4])
        yield 14
        z256 = _csq(z[128])
        put(6, z[4], z256)
        z512 = _csq(z256)
        put(8, z512, z512)
        q258 = _cmul(z[2], z256)
        q516 = _csq(q258)
        put(4, _cmul(w, q258), _cmul(w, q516))
        p1032 = _cmul(w, _csq(q516))
        put(7, p1032, _cmul(p1032, z256))
        yield 18

    def kgen_tables(buf, c, h):
        def seed(slot):
            return tuple(seed_v[6 * buf + 2 * c + h, 2 * slot + i] for i in range(2))

        def emit(ref, i, v0, v1):
            (re0, im0), (re1, im1) = v0, v1
            rows = pl.ds(16 * i, 16)
            if c < 2:
                ref[12 * buf + 3 * (2 * c + h), rows, :] = _pack(re0, re1)
                ref[12 * buf + 3 * (2 * c + h) + 1, rows, :] = _pack(im0, im1)
            else:
                im0, im1 = pltpu.roll(im0, 64, 1), pltpu.roll(im1, 64, 1)
                ref[12 * buf + 3 * h + 2, rows, :] = _pack(
                    jnp.where(left, re0, im0), jnp.where(left, re1, im1))
                ref[12 * buf + 3 * (2 + h) + 2, rows, :] = _pack(
                    jnp.where(left, im0, re0), jnp.where(left, im1, re1))

        for ref, first, n in ((rhs_all, 0, 8), (lhs_all, 2, 2)):
            v, m = seed(first), seed(first + 1)
            for i in range(n):
                v1 = _cmul(v, m)
                emit(ref, i, v, v1)
                yield 4
                if i + 1 < n:
                    v = _cmul(v1, m)
        v, m = seed(4), seed(6)
        v1 = _cmul(v, seed(5))
        emit(lhs_all, 2, v, v1)
        emit(lhs_all, 3, _cmul(v, m), _cmul(v1, m))
        v = seed(7)
        emit(lhs_all, 4, v, _cmul(v, seed(8)))
        yield 4

    def kgen_contract(step, buf):
        r0 = pl.multiple_of(step * 16, 16)
        diag = (lane & ~3) | (sub & 3)
        slot = lane & 3
        tiles = []
        for grp in range(2):
            w = []
            for h in range(2):
                idx = [12 * buf + 3 * (2 * grp + h) + i for i in range(3)]
                o = lax.dot_general(_cat(lhs_all, idx), _cat(rhs_all, idx), _NT_DIMS,
                                    preferred_element_type=F32)
                yield 60
                p = [_lane_gather(o[8 * i:8 * i + 8], diag) for i in range(10)]

                def sel4(v):
                    return jnp.where(slot < 2, jnp.where(slot == 0, v[0], v[1]),
                                     jnp.where(slot == 2, v[2], v[3]))
                w.append((sel4(p[0:4]), sel4(p[4:8]),
                          jnp.where((slot & 1) == 0, p[8], p[9])))
            hi = [jnp.where(upper, a, b) for a, b in zip(*w)]
            lo = [pltpu.roll(jnp.where(upper, b, a), 4, 0) for a, b in zip(*w)]
            even = (lane & 4) == 0
            tiles.append((
                jnp.where(even, hi[0], pltpu.roll(lo[0], 4, 1)),
                jnp.where(even, pltpu.roll(hi[0], 124, 1), lo[0]),
                hi[1], lo[1], jnp.where(slot < 2, hi[2], lo[2])))
        for t in range(5):
            kd_v[t, pl.ds(r0, 16), :] = _pack(tiles[0][t], tiles[1][t])

    def seeds(s0, *offs):
        return [(kgen_seeds, (jnp.minimum(s0 + i, D // 16 - 1), i % KB, c), 88)
                for i in offs for c in range(3)]

    def tables(*offs):
        return [(kgen_tables, (i % KB, c, h), 44)
                for i in offs for c in range(3) for h in range(2)]

    def contract(s0, *offs):
        return [(kgen_contract, (s0 + i, i % KB), 240) for i in offs]

    def u_dft(c, t):
        rows = pl.ds(pl.multiple_of(c * (T // 2), T // 2), T // 2)
        for r in range(0, T, 64):
            re, im = (jnp.dot(_bf16(fu_ref[pl.ds((o + r) // 2, 32), :]), _bf16(u_w[t, rows, :]),
                              preferred_element_type=F32) for o in (0, T))
            uh_v[t, c, r:r + 64, :] = re
            uh_v[t, c, T + r:T + r + 64, :] = im
            uh_v[t, c, 2 * T + r:2 * T + r + 64, :] = re + im
            yield 32

    wraw_w = wraw_v.bitcast(jnp.int32)
    res5 = lane - 5 * ((lane * 205) >> 10)

    def reorder_qkv(j, p):
        col = ((lane & (H - 1)) * DH + 5 * (lane >> 5) + j) & 127
        for i in range(D // 16):
            rows = pl.ds(8 * i, 8)
            acc = wraw_w[NT * p, rows, :]
            for t in range(1, NT):
                acc = jnp.where(res5 == (j - 128 * t) % 5,
                                wraw_w[NT * p + t, rows, :], acc)
            w_v[NT * p + j, rows, :] = _lane_gather(acc, col)
            if i % 8 == 7:
                yield 0.2

    def reorder_out(t):
        wof_v[t, 0:D, :] = woraw_v[:, 128 * t:128 * t + 128].astype(F32)
        for j in range(NT):
            for i in range(4):
                r = 128 * j + H * i
                wo_v[t, r:r + H, :] = wof_v[t, pl.ds(j + 5 * i, H, stride=DH), :].astype(BF16)
            yield 0.2

    def keep_halo(ref):
        for t in range(NT):
            ref[t, 0:HALO, :] = ref[t, RB:RB + HALO, :]

    def project(blk, p, g, first, tiles=range(NT)):
        ref, r0 = ((q_v, 0), (k_v, HALO), (v_v, HALO))[p]
        if p > 0 and g == 0 and not first:
            keep_halo(ref)

        def rows(m):
            return pl.ds(pl.multiple_of(blk * (RB // 2) + m * (MM // 2), MM // 2), MM // 2)

        def tail(t):
            for m in range(4 * g, 4 * g + 4):
                ref[t, pl.ds(r0 + m * MM, MM), :] = jnp.dot(
                    _cat(x_w, [4], rows(m)), _bf16(w_v[NT * p + t, 256:320]),
                    preferred_element_type=F32)

        def main(t, m):
            dst = pl.ds(r0 + m * MM, MM)
            val = ref[t, dst, :] + jnp.dot(
                _cat(x_w, range(4), rows(m)), _bf16(w_v[NT * p + t, 0:256]),
                preferred_element_type=F32)
            ref[t, dst, :] = val * (DH ** -0.5 * LOG2E) if p == 0 else val
            if p > 0 and first and m == 0:
                ref[t, 0:HALO, :] = jnp.broadcast_to(val[0:1], (HALO, 128))

        for t in tiles:
            tail(t)
            yield MM
            for m in range(4 * g, 4 * g + 4):
                main(t, m)
                yield MM

    def projects(blk, p, first=False):
        return [(project, (blk, p, g, first), MM * 25) for g in range(RB // MM // 4)]

    def logits(i, first):
        for w in range(WIN // 2):
            a = HALO + 8 * i - DIL * w
            keys = [k_v[t, a:a + 8, :] for t in range(NT)]
            for r, ww in ((8 * i, w), (8 * i + 8, w + WIN // 2)):
                if not 0 <= r < RB:
                    continue
                s = q_v[0, r:r + 8, :] * keys[0]
                for t in range(1, NT):
                    s = s + q_v[t, r:r + 8, :] * keys[t]
                if first and r < DIL * ww:
                    s = jnp.where(sub >= DIL * ww - r, s, -0.25e9 * LOG2E)
                e_v[ww, r:r + 8, :] = s
            yield 0.25

    def fold(i):
        for w in range(WIN):
            s = e_v[w, 8 * i:8 * i + 8, :]
            e_v[w, 8 * i:8 * i + 8, :] = s + pltpu.roll(s, 64, 1)

    def weights(i):
        lg = []
        for w in range(WIN):
            s = e_v[w, 8 * i:8 * i + 8, :]
            lg.append(s + pltpu.roll(s, 32, 1))
        m = lg[0]
        for s in lg[1:]:
            m = jnp.maximum(m, s)
        den = None
        for w in range(WIN):
            e = jnp.exp2(lg[w] - m)
            p_v[w, 8 * i:8 * i + 8, :] = e
            den = e if den is None else den + e
        p_v[WIN, 8 * i:8 * i + 8, :] = 1.0 / den

    def mix(blk, i):
        rows = pl.ds(pl.multiple_of(blk * RB + 16 * i, 16), 16)
        res = []
        for r in (16 * i, 16 * i + 8):
            e = [p_v[w, r:r + 8, :] for w in range(WIN + 1)]
            for t in range(NT):
                acc = None
                for w in range(WIN):
                    a = HALO + r - DIL * w
                    term = e[w] * v_v[t, a:a + 8, :]
                    acc = term if acc is None else acc + term
                res.append(acc * e[WIN])
                if len(res) > NT:
                    o_v[t, rows, :] = _pack(res[t], res[-1])
                yield 0.1

    NI = RB // 16
    all_weights = []
    for i in range(2 * NI + 16):
        if i < 2 * NI:
            all_weights.append((fold, (i,), 0.5))
        if i >= 16:
            all_weights.append((weights, (i - 16,), 1))

    def all_logits(first):
        return [(logits, (i, first), 1) for i in range(-1, 2 * NI)]

    def mixes(blk):
        return [(mix, (blk, i), 1) for i in range(NI)]

    def u_dfts(c):
        return [(u_dft, (c + i, t), 64) for i in range(RB // T) for t in range(NT)]

    def reorders(p):
        return [(reorder_qkv, (j, p), 1) for j in range(NT)]

    q, k, v = (projects(0, p, True) for p in range(3))
    wait(groups[0])
    _weave([(ssm_setup, (0,), 300)] + seeds(0, 0, 1, 2, 3))
    wait(groups[1])
    _weave(reorders(0))
    wait(groups[2])
    _weave(tables(0, 1), seeds(0, 4, 5), q[:1])
    wait(groups[3])
    _weave(seeds(0, 6), [(project, (0, 0, 1, True, range(2)), MM * 10)])
    wait(groups[4])
    _weave(reorders(1), [(project, (0, 0, 1, True, range(2, NT)), MM * 15)])
    _weave(seeds(0, 7), k[:1])
    wait(groups[5])
    _weave(reorders(2), tables(2, 3), k[1:])
    wait(groups[6])
    region(lambda: _weave([(ssm_setup, (t,), 1) for t in range(1, NT)], all_logits(True), v))
    wait(groups[7])

    def attn_body(blk, carry):
        @pl.when(blk == 2)
        def _():
            wait(groups[8])
            start(groups[9])

        s0 = KB * (blk - 1)
        region(lambda: _weave(
            tables(4, 5, 6, 7) + seeds(s0, *range(8, 11)), all_weights,
            contract(s0, 0, 1, 2, 3) + projects(blk, 0)))
        region(lambda: _weave(
            seeds(s0, *range(11, 16)) + tables(8, 9, 10), mixes(blk - 1),
            contract(s0, 4, 5) + projects(blk, 1), u_dfts(4 * blk - 4)))
        _weave(seeds(s0, *range(16, 19)) + tables(11, 12, 13, 14), all_logits(False),
               contract(s0, 6, 7, 8, 9, 10) + projects(blk, 2))
        return carry

    lax.fori_loop(1, L // RB, attn_body, 0)

    wait(groups[9])
    ch, yh = (ch0_v, ch1_v), (yh0_v, yh1_v)

    out_copies = []

    def write_out(part, t, r0=0, r1=L):
        c0 = D * part + 128 * t
        out_copies.append(pltpu.make_async_copy(
            (ya_v, yb_v)[part].at[t, r0:r1], out_hbm.at[0, r0:r1, c0:c0 + 128], out_sem))
        out_copies[-1].start()

    def k_dft(t, j):
        ta, tb, pick = _G_TILES[j]
        kd_w = kd_v.bitcast(jnp.int32)
        vals = kd_w[ta, 64 * t:64 * t + 64, :]
        if pick:
            vals = jnp.where(pick(_iota((64, 128), 1)), vals, kd_w[tb, 64 * t:64 * t + 64, :])
        for r in range(0, T, 64):
            re, im = (lax.dot_general(_bf16(g_v[j, pl.ds((o + r) // 2, 32), :]), _bf16(vals),
                                      _NT_DIMS, preferred_element_type=F32) for o in (0, T))
            if j < _SPLIT - 1:
                acc_v[j, r:r + 64, :], acc_v[j, T + r:T + r + 64, :] = re, im
            if 0 < j < _SPLIT:
                pre, pim = acc_v[j - 1, r:r + 64, :], acc_v[j - 1, T + r:T + r + 64, :]
                re, im = (re - pim, im + pre) if r == 0 else (re + pim, im - pre)
            ch[t % 2][j, r:r + 64, :] = re
            ch[t % 2][j, T + r:T + r + 64, :] = im - re
            ch[t % 2][j, 2 * T + r:2 * T + r + 64, :] = im + re
            yield 32

    def block_conv(t, r):
        tmp = tmp_v.at[r % 2]
        nh = NB // 2
        for part in range(3):
            for phase, (pc, pu) in enumerate(((0, 2), (1, 0), (2, 1))):
                def fetch(get):
                    return [get(2 * c + part) if part < 2 else get(2 * c) + get(2 * c + 1)
                            for c in range(nh)]
                f = fetch(lambda c: ch[t % 2][c, pl.ds(T * pc + 8 * r, 8), :])
                g = fetch(lambda c: uh_v[t, c, pl.ds(T * pu + 8 * r, 8), :])
                for n0 in range(0, nh, CG):
                    acc = {n: tmp[0, 0, n] if phase else None for n in range(n0, n0 + CG)}
                    for j in range(n0 + CG):
                        for n in range(max(n0, j), n0 + CG):
                            term = f[j] * g[n - j]
                            acc[n] = (term if acc[n] is None else
                                      acc[n] - term if phase == 2 else acc[n] + term)
                    for n in acc:
                        if phase == 0:
                            tmp[0, 0, n] = acc[n]
                        elif part < 2:
                            tmp[phase, part, n] = acc[n]
                        else:
                            odd = acc[n] - tmp[phase, 0, n] - tmp[phase, 1, n]
                            even = tmp[phase, 0, n]
                            if n:
                                even = even + tmp[phase, 1, n - 1]
                            if phase == 1:
                                tmp[0, 1, n], tmp[0, 2, n] = even, odd
                            else:
                                rows = pl.ds(16 * r, 16)
                                yh[t % 2][2 * n, rows, :] = _pack(even, tmp[0, 1, n])
                                yh[t % 2][2 * n + 1, rows, :] = _pack(odd, tmp[0, 2, n])
                    yield (6 if n0 == 0 else 11) + (5 if part == 2 else 0)

    def inv_dft(t, c):
        for r in range(0, T, 64):
            y = jnp.dot(_cat(fi_ref, range(2), pl.ds(r // 2, 32)), _cat(yh[t % 2], [c]),
                        preferred_element_type=F32)
            rows = pl.ds(T * c + r, 64)
            ya_v[t, rows, :] = (y + u_v[t, rows, :].astype(F32) * skip_v[t]).astype(BF16)
            yield 32

    def out_proj(n):
        t, c = n // 4, n % 4
        wo_w = wo_v.bitcast(jnp.int32)
        for m in range(512 // MM):
            acc_v[4 + c, m * MM:(m + 1) * MM, :] = jnp.dot(
                _cat(o_v, [4], pl.ds(256 * c + m * MM // 2, MM // 2)),
                _bf16(wo_w[t, 256:320]), preferred_element_type=F32)
            yield MM // 4
        for m in range(512 // MM):
            yb_v[t, pl.ds(512 * c + m * MM, MM), :] = (
                acc_v[4 + c, m * MM:(m + 1) * MM, :] + jnp.dot(
                    _cat(o_v, range(4), pl.ds(256 * c + m * MM // 2, MM // 2)),
                    _bf16(wo_w[t, 0:256]), preferred_element_type=F32)).astype(BF16)
            yield MM

    def k_dfts(t, js):
        return [(k_dft, (t, j), 64) for j in js]

    s0 = KB * (L // RB - 1)
    region(lambda: _weave(
        tables(4), all_weights, [(reorder_out, (t,), 1) for t in range(NT)],
        contract(s0, 0, 1, 2, 3) + k_dfts(0, range(NB)), u_dfts(NB - 4)))
    region(lambda: _weave(
        tables(5, 6), mixes(L // RB - 1),
        contract(s0, 4) + [(out_proj, (n,), 640) for n in range(3)]))
    write_out(1, 0, 0, 1536)
    plan = [(0, range(NB), range(3, 6)), (1, range(NB), range(6, 9)),
            (2, range(NB), range(9, 12)), (3, range(NB), range(12, 15)),
            (4, range(0, 11), range(15, 18)), (4, range(11, NB), range(18, 20))]
    for t, freqs, chunks in plan:
        head = freqs[0] == 0
        region(lambda: _weave(
            [(block_conv, (t, i), 183) for i in freqs],
            ([(inv_dft, (t - 1, c), 64) for c in range(NB)] if t > 0 and head else
             contract(s0, 5, 6) if t == 0 else [])
            + [(out_proj, (n,), 640) for n in chunks],
            k_dfts(t + 1, range(NB)) if t + 1 < NT else []))
        if t > 0 and head:
            write_out(0, t - 1)
        for n in chunks:
            write_out(1, n // 4, 512 * (n % 4), 512 * (n % 4) + 512)
    for c0, c1 in ((0, 4), (4, 8), (8, 12), (12, 16)):
        _weave([(inv_dft, (NT - 1, c), 64) for c in range(c0, c1)])
        write_out(0, NT - 1, T * c0, T * c1)
    wait(out_copies)


@jax.jit
def pallas_concat_heads__ssm_conv_s4__sliding_local_dilated__prompt_kernel(
    A_u: jax.Array,
    A_A_re: jax.Array,
    A_A_im: jax.Array,
    A_B_re: jax.Array,
    A_B_im: jax.Array,
    A_C_re: jax.Array,
    A_C_im: jax.Array,
    A_log_dt: jax.Array,
    A_Dskip: jax.Array,
    B_x: jax.Array,
    B_wqkv: jax.Array,
    B_wo: jax.Array,
):
    hbm = pl.BlockSpec(memory_space=pl.ANY)
    I32 = jnp.int32
    return pl.pallas_call(
        _kernel,
        out_shape=jax.ShapeDtypeStruct((1, L, 2 * D), BF16),
        in_specs=[hbm] * 15 + [pl.BlockSpec(memory_space=pltpu.SMEM)],
        out_specs=hbm,
        scratch_shapes=[
            pltpu.VMEM(_FU.shape, I32),
            pltpu.VMEM(_FI.shape, I32),
            pltpu.VMEM((6, N, D), BF16),
            pltpu.VMEM((NT, L, 128), BF16),
            pltpu.VMEM((NT, L, 128), BF16),
            pltpu.VMEM((3 * NT, D, 128), BF16),
            pltpu.VMEM((D, D), BF16),
            pltpu.VMEM(_G.shape, I32),
            pltpu.VMEM((3 * NT, D // 2, 128), I32),
            pltpu.VMEM((NT, D, 128), BF16),
            pltpu.VMEM((NT, D + 32, 128), F32),
            pltpu.VMEM((6, D, 128), F32),
            pltpu.VMEM((KB * 6, 18, 8, 128), F32),
            pltpu.VMEM((KB * 12, 80, 128), BF16),
            pltpu.VMEM((KB * 12, 128, 128), BF16),
            pltpu.VMEM((5, D, 128), BF16),
            pltpu.VMEM((NT, RB, 128), F32),
            pltpu.VMEM((NT, HALO + RB, 128), F32),
            pltpu.VMEM((NT, HALO + RB, 128), F32),
            pltpu.VMEM((WIN, RB, 128), F32),
            pltpu.VMEM((WIN + 1, RB, 128), F32),
            pltpu.VMEM((NT, L, 128), BF16),
            pltpu.VMEM((8, 512, 128), F32),
            pltpu.VMEM((2, 3, 3, NB // 2, 8, 128), F32),
            pltpu.VMEM((NT, NB, 3 * T, 128), F32),
            pltpu.VMEM((NB, 3 * T, 128), F32),
            pltpu.VMEM((NB, 3 * T, 128), F32),
            pltpu.VMEM((NB, 2 * T, 128), BF16),
            pltpu.VMEM((NB, 2 * T, 128), BF16),
            pltpu.VMEM((NT, L, 128), BF16),
            pltpu.VMEM((NT, L, 128), BF16),
            pltpu.VMEM((NT, 1, 128), F32),
            pltpu.VMEM((D,), BF16),
            pltpu.VMEM((D,), BF16),
            pltpu.SemaphoreType.DMA((10,)),
            pltpu.SemaphoreType.DMA(()),
        ],
        compiler_params=pltpu.CompilerParams(vmem_limit_bytes=100 * 1024 * 1024),
        name="s4_attn",
    )(A_u, A_A_re.T, A_A_im.T, A_B_re.T, A_B_im.T, A_C_re.T, A_C_im.T,
      A_log_dt, A_Dskip, B_x, B_wqkv, B_wo, _G, _FU, _FI, np.ones((1,), np.int32))
```
